```python
import os as _os
_os.environ.setdefault("JAX_PLATFORMS", "cpu")
import jax
import jax.numpy as jnp

def _softmax(x, axis=-1):
    return jax.nn.softmax(x, axis=axis)
def _gelu(x):
    return jax.nn.gelu(x, approximate=True)
def _silu(x):
    return jax.nn.silu(x)
def _sigmoid(x):
    return jax.nn.sigmoid(x)
def _layernorm(x, axis=-1, eps=1e-5):
    m = jnp.mean(x, axis=axis, keepdims=True)
    v = jnp.var(x, axis=axis, keepdims=True)
    return (x - m) / jnp.sqrt(v + eps)
def _scatter_add(tgt, idx, src, axis=0):
    return tgt.at[idx].add(src)
def _segment_sum(src, seg, n):
    return jax.ops.segment_sum(src, seg, n)
class _Rng:
    def __init__(self, key):
        self._k = key
    def _next(self):
        self._k, sub = jax.random.split(self._k)
        return sub
    def normal(self, shape):
        return jax.random.normal(self._next(), shape, dtype=jnp.bfloat16)
    def randint(self, lo, hi, shape):
        return jax.random.randint(self._next(), shape, lo, hi, dtype=jnp.int32)
    def uniform(self, shape, lo=0.0, hi=1.0):
        return jax.random.uniform(self._next(), shape, jnp.bfloat16, lo, hi)
    def permutation(self, n):
        return jax.random.permutation(self._next(), n)


kernel_name = 'sequential_preLN__softmax_full_mha__dense_activation_gelu__prompt'

def setup_inputs():
    _rng = _Rng(jax.random.key(int.from_bytes(__import__("os").urandom(4), "little")))
    _w = (lambda a: (lambda t: t.astype(jnp.bfloat16) if jnp.issubdtype(t.dtype, jnp.floating) else t)(jnp.asarray(a)))
    def _A_setup():
        B, S, D = 1, 2048, 640
        return {
            "x": _w((lambda *s: _rng.normal(s) * 0.05)(B, S, D)),
            "wqkv": _w((lambda *s: _rng.normal(s) * 0.05)(D, 3 * D)),
            "wo": _w((lambda *s: _rng.normal(s) * 0.05)(D, D)),
        }
    _A_in = _A_setup()

    def _B_setup():
        B, S, D, F = 1, 2048, 640, 1536
        return {
            "x": _w((lambda *s: _rng.normal(s) * 0.05)(B, S, D)),
            "w1": _w((lambda *s: _rng.normal(s) * 0.4)(D, F) * (D ** -0.5)),
            "b1": _w((lambda *s: _rng.normal(s) * 0.4)(F) * 0.01),
            "w2": _w((lambda *s: _rng.normal(s) * 0.4)(F, D) * (F ** -0.5)),
            "b2": _w((lambda *s: _rng.normal(s) * 0.05)(D) * 0.01),
        }
    _B_in = _B_setup()

    return {
        "A_x": _A_in["x"],
        "A_wqkv": _A_in["wqkv"],
        "A_wo": _A_in["wo"],
        "B_x": _B_in["x"],
        "B_w1": _B_in["w1"],
        "B_b1": _B_in["b1"],
        "B_w2": _B_in["w2"],
        "B_b2": _B_in["b2"],
    }

def reference(A_x, A_wqkv, A_wo, B_x, B_w1, B_b1, B_w2, B_b2):
    def _A_ref(x, wqkv, wo):
        B, S, D = x.shape
        H = 32; Dh = D // H
        qkv = (lambda x, *d: x.transpose(*d))((x @ wqkv).reshape(B, S, 3, H, Dh), 2, 0, 3, 1, 4)
        q, k, v = qkv[0], qkv[1], qkv[2]
        scale = Dh ** -0.5
        scores = jnp.einsum("bhqd,bhkd->bhqk", q, k) * scale
        p = _softmax(scores, axis=-1)
        o = jnp.einsum("bhqk,bhkd->bhqd", p, v)
        return (lambda x, *d: x.transpose(*d))(o, 0, 2, 1, 3).reshape(B, S, D) @ wo

    def _B_ref(x, w1, b1, w2, b2):
        h = jnp.einsum("bsd,df->bsf", x, w1) + b1
        h = _gelu(h)
        return jnp.einsum("bsf,fd->bsd", h, w2) + b2

    x = A_x
    h = x + _A_ref(_layernorm(x, axis=-1), A_wqkv, A_wo)
    h2 = h + _B_ref(_layernorm(h, axis=-1), B_w1, B_b1, B_w2, B_b2)
    return h2
```

```python
import math

import jax
import jax.numpy as jnp
import jax.experimental.pallas as pl
import jax.experimental.pallas.tpu as pltpu

_H = 32
_EPS = 1e-5
_RC = 512
_NQ = 512
_KC = 128
_FC = 256

_F32 = jnp.float32
_BF16 = jnp.bfloat16


def _dot(a, b):
    return jnp.dot(a, b, preferred_element_type=_F32)


def _dot_nt(a, b):
    return jax.lax.dot_general(
        a, b, (((1,), (1,)), ((), ())), preferred_element_type=_F32)


def _layernorm(x):
    d = x - jnp.mean(x, axis=-1, keepdims=True)
    v = jnp.mean(d * d, axis=-1, keepdims=True)
    return d * jax.lax.rsqrt(v + _EPS)


def _gelu(x):
    c = math.sqrt(2.0 / math.pi)
    return x * (0.5 * (1.0 + jnp.tanh(c * (x + 0.044715 * (x * x * x)))))


def _kernel(x_hbm, wqkv_hbm, wo_hbm, w1_hbm, b1_hbm, w2_hbm, b2_hbm, out_hbm,
            x_v, wk_v, wq_v, wv_v, wo_v, w1_v, b1_v, w2_v, b2_v, out_v,
            xn_s, k_s, q_s, v_s, sa, sb, o_s, sems):
    S, D = x_v.shape
    dh = D // _H
    vm = v_s.shape[1]
    nrc, nqb, nkc, nfc = S // _RC, S // _NQ, S // _KC, S // _FC

    sem_id = iter(range(sems.shape[0]))

    def copy(src, dst):
        return pltpu.make_async_copy(src, dst, sems.at[next(sem_id)])

    x_cp = [copy(x_hbm.at[0, pl.ds(c * _RC, _RC)], x_v.at[pl.ds(c * _RC, _RC)])
            for c in range(nrc)]
    wq_cp = copy(wqkv_hbm.at[:, pl.ds(0, D)], wq_v)
    wk_cp = copy(wqkv_hbm.at[:, pl.ds(D, D)], wk_v)
    wv_cp = copy(wqkv_hbm.at[:, pl.ds(2 * D, D)], wv_v)
    late_cp = [copy(wo_hbm, wo_v), copy(w1_hbm, w1_v), copy(b1_hbm, b1_v),
               copy(w2_hbm, w2_v), copy(b2_hbm, b2_v)]
    out_cp = [copy(out_v.at[pl.ds(c * _FC, _FC)], out_hbm.at[0, pl.ds(c * _FC, _FC)])
              for c in range(nfc)]

    x_cp[0].start()
    wk_cp.start()
    x_cp[0].wait()
    wk_cp.wait()
    for cp in x_cp[1:] + [wq_cp, wv_cp]:
        cp.start()
    for c in range(nrc):
        if c == 1:
            for cp in x_cp[1:]:
                cp.wait()
        rows = pl.ds(c * _RC, _RC)
        xn = _layernorm(x_v[rows, :].astype(_F32)).astype(_BF16)
        xn_s[rows, :] = xn
        k = _dot(xn, wk_v[...]).astype(_BF16)
        for h in range(_H):
            k_s[h, rows, :] = k[:, h * dh:(h + 1) * dh]
    wq_cp.wait()
    wv_cp.wait()
    for cp in late_cp:
        cp.start()
    wq_t = wq_v[...].T
    wv_t = wv_v[...].T
    qscale = dh ** -0.5 * math.log2(math.e)
    row = jax.lax.broadcasted_iota(jnp.int32, (vm - dh, _RC), 0)
    v_tail = jnp.where(row == 0, 1.0, 0.0).astype(_F32)
    for c in range(nrc):
        cols = pl.ds(c * _RC, _RC)
        xn = xn_s[cols, :]
        qt = _dot_nt(wq_t, xn) * qscale
        vt = _dot_nt(wv_t, xn)
        for h in range(_H):
            q_s[h, :, cols] = qt[h * dh:(h + 1) * dh, :].astype(_BF16)
            v_s[h, :, cols] = jnp.concatenate(
                [vt[h * dh:(h + 1) * dh, :], v_tail], axis=0)

    def step(nxt, cur):
        m = acc = None
        if nxt is not None:
            h1, qb1, s1 = nxt
            q = q_s[h1, :, pl.ds(pl.multiple_of(qb1 * _NQ, _NQ), _NQ)]
        if cur is not None:
            h0, s0, m0 = cur
        for c in range(nkc):
            keys = pl.ds(c * _KC, _KC)
            if nxt is not None:
                s = _dot(k_s[h1, keys, :], q)
                s1[keys, :] = s
                mm = jnp.max(s.reshape(_KC // 8, 8, _NQ), axis=0)
                m = mm if m is None else jnp.maximum(m, mm)
            if cur is not None:
                p = jnp.exp2(s0[keys, :] - m0).astype(_BF16)
                r = _dot(v_s[h0, :, keys], p)
                acc = r if acc is None else acc + r
        if m is not None:
            m = jnp.max(m, axis=0, keepdims=True)
        if acc is not None:
            acc = acc[:dh] / acc[dh:dh + 1]
        return m, acc

    hp = _H // 2

    def pair(j, m, last=False):
        qb, g = j // hp, j % hp
        m, o0 = step((2 * g + 1, qb, sb), (2 * g, sa, m))
        j1 = j + 1
        nxt = None if last else (2 * (j1 % hp), j1 // hp, sa)
        m, o1 = step(nxt, (2 * g + 1, sb, m))
        o_s[g, :, pl.ds(pl.multiple_of(qb * _NQ, _NQ), _NQ)] = (
            jnp.concatenate([o0, o1], axis=0))
        return m

    m, _ = step((0, 0, sa), None)
    m = jax.lax.fori_loop(0, nqb * hp - 1, pair, m)
    pair(nqb * hp - 1, m, last=True)

    for cp in late_cp:
        cp.wait()
    b1 = b1_v[...].astype(_F32).reshape(1, -1)
    b2 = b2_v[...].astype(_F32).reshape(1, -1)
    for c in range(nfc):
        rows = pl.ds(c * _FC, _FC)
        ot = o_s[:, :, rows].reshape(D, _FC)
        o = ot.T.astype(_BF16)
        h = x_v[rows, :].astype(_F32) + _dot(o, wo_v[...])
        hn = _layernorm(h).astype(_BF16)
        a = _gelu(_dot(hn, w1_v[...]) + b1).astype(_BF16)
        out_v[rows, :] = (h + (_dot(a, w2_v[...]) + b2)).astype(out_v.dtype)
        out_cp[c].start()
    for cp in out_cp:
        cp.wait()


@jax.jit
def pallas_sequential_preLN__softmax_full_mha__dense_activation_gelu__prompt_kernel(
    A_x: jax.Array,
    A_wqkv: jax.Array,
    A_wo: jax.Array,
    B_x: jax.Array,
    B_w1: jax.Array,
    B_b1: jax.Array,
    B_w2: jax.Array,
    B_b2: jax.Array,
):
    del B_x
    _, S, D = A_x.shape
    F = B_w1.shape[1]
    dh = D // _H
    vm = -(-(dh + 1) // 8) * 8
    dt = A_x.dtype
    any_spec = pl.BlockSpec(memory_space=pl.ANY)
    return pl.pallas_call(
        _kernel,
        out_shape=jax.ShapeDtypeStruct(A_x.shape, dt),
        in_specs=[any_spec] * 7,
        out_specs=any_spec,
        scratch_shapes=[
            pltpu.VMEM((S, D), dt),
            pltpu.VMEM((D, D), dt),
            pltpu.VMEM((D, D), dt),
            pltpu.VMEM((D, D), dt),
            pltpu.VMEM((D, D), dt),
            pltpu.VMEM((D, F), dt),
            pltpu.VMEM((F,), dt),
            pltpu.VMEM((F, D), dt),
            pltpu.VMEM((D,), dt),
            pltpu.VMEM((S, D), dt),
            pltpu.VMEM((S, D), _BF16),
            pltpu.VMEM((_H, S, dh), _BF16),
            pltpu.VMEM((_H, dh, S), _BF16),
            pltpu.VMEM((_H, vm, S), _F32),
            pltpu.VMEM((S, _NQ), _F32),
            pltpu.VMEM((S, _NQ), _F32),
            pltpu.VMEM((_H // 2, 2 * dh, S), _F32),
            pltpu.SemaphoreType.DMA((S // _RC + 8 + S // _FC,)),
        ],
        compiler_params=pltpu.CompilerParams(vmem_limit_bytes=100 * 2**20),
    )(A_x, A_wqkv, A_wo, B_w1, B_b1, B_w2, B_b2)
```

```python
import math

import jax
import jax.numpy as jnp
import jax.experimental.pallas as pl
import jax.experimental.pallas.tpu as pltpu

_H = 32
_EPS = 1e-5
_RC = 512
_NQ = 512
_KC = 128
_FC = 256

_F32 = jnp.float32
_BF16 = jnp.bfloat16


def _dot(a, b):
    return jnp.dot(a, b, preferred_element_type=_F32)


def _dot_nt(a, b):
    return jax.lax.dot_general(
        a, b, (((1,), (1,)), ((), ())), preferred_element_type=_F32)


def _layernorm(x):
    d = x - jnp.mean(x, axis=-1, keepdims=True)
    v = jnp.mean(d * d, axis=-1, keepdims=True)
    return d * jax.lax.rsqrt(v + _EPS)


def _gelu(x):
    c = math.sqrt(2.0 / math.pi)
    return x * (0.5 * (1.0 + jnp.tanh(c * (x + 0.044715 * (x * x * x)))))


def _kernel(x_hbm, wqkv_hbm, wo_hbm, w1_hbm, b1_hbm, w2_hbm, b2_hbm, out_hbm,
            x_v, wk_v, wq_v, wv_v, wo_v, w1_v, b1_v, w2_v, b2_v, out_v,
            xn_s, kall_s, k_s, q_s, v_s, sa, sb, o_s, sems):
    S, D = x_v.shape
    dh = D // _H
    vm = v_s.shape[1]
    nrc, nqb, nkc, nfc = S // _RC, S // _NQ, S // _KC, S // _FC

    sem_id = iter(range(sems.shape[0]))

    def copy(src, dst):
        return pltpu.make_async_copy(src, dst, sems.at[next(sem_id)])

    x_cp = [copy(x_hbm.at[0, pl.ds(c * _RC, _RC)], x_v.at[pl.ds(c * _RC, _RC)])
            for c in range(nrc)]
    wq_cp = copy(wqkv_hbm.at[:, pl.ds(0, D)], wq_v)
    wk_cp = copy(wqkv_hbm.at[:, pl.ds(D, D)], wk_v)
    wv_cp = copy(wqkv_hbm.at[:, pl.ds(2 * D, D)], wv_v)
    late_cp = [copy(wo_hbm, wo_v), copy(w1_hbm, w1_v), copy(b1_hbm, b1_v),
               copy(w2_hbm, w2_v), copy(b2_hbm, b2_v)]
    out_cp = [copy(out_v.at[pl.ds(c * _FC, _FC)], out_hbm.at[0, pl.ds(c * _FC, _FC)])
              for c in range(nfc)]

    x_cp[0].start()
    wk_cp.start()
    x_cp[0].wait()
    wk_cp.wait()
    for cp in x_cp[1:] + [wq_cp, wv_cp]:
        cp.start()
    for c in range(nrc):
        if c == 1:
            for cp in x_cp[1:]:
                cp.wait()
        rows = pl.ds(c * _RC, _RC)
        xn = _layernorm(x_v[rows, :].astype(_F32)).astype(_BF16)
        xn_s[rows, :] = xn
        kall_s[rows, :] = _dot(xn, wk_v[...]).astype(_BF16)
    wq_cp.wait()
    wv_cp.wait()
    for cp in late_cp:
        cp.start()
    wq_t = wq_v[...].T
    wv_t = wv_v[...].T
    qscale = dh ** -0.5 * math.log2(math.e)
    row = jax.lax.broadcasted_iota(jnp.int32, (vm - dh, _RC), 0)
    v_tail = jnp.where(row == 0, 1.0, 0.0).astype(_F32)
    first = jax.lax.broadcasted_iota(jnp.int32, (2 * dh, _RC), 0) < dh
    for c in range(nrc):
        cols = pl.ds(c * _RC, _RC)
        xn = xn_s[cols, :]
        qt = _dot_nt(wq_t, xn) * qscale
        vt = _dot_nt(wv_t, xn)
        k = kall_s[cols, :]
        for g in range(_H // 2):
            k_s[g, cols, :] = k[:, 2 * g * dh:2 * (g + 1) * dh]
            qg = qt[2 * g * dh:2 * (g + 1) * dh, :]
            q_s[2 * g, :, cols] = jnp.where(first, qg, 0.0).astype(_BF16)
            q_s[2 * g + 1, :, cols] = jnp.where(first, 0.0, qg).astype(_BF16)
        for h in range(_H):
            v_s[h, :, cols] = jnp.concatenate(
                [vt[h * dh:(h + 1) * dh, :], v_tail], axis=0)

    def step(nxt, cur):
        m = acc = None
        if nxt is not None:
            h1, qb1, s1 = nxt
            q = q_s[h1, :, pl.ds(pl.multiple_of(qb1 * _NQ, _NQ), _NQ)]
        if cur is not None:
            h0, s0, m0 = cur
        for c in range(nkc):
            keys = pl.ds(c * _KC, _KC)
            if nxt is not None:
                s = _dot(k_s[h1 // 2, keys, :], q)
                s1[keys, :] = s
                mm = jnp.max(s.reshape(_KC // 8, 8, _NQ), axis=0)
                m = mm if m is None else jnp.maximum(m, mm)
            if cur is not None:
                p = jnp.exp2(s0[keys, :] - m0).astype(_BF16)
                r = _dot(v_s[h0, :, keys], p)
                acc = r if acc is None else acc + r
        if m is not None:
            m = jnp.max(m, axis=0, keepdims=True)
        if acc is not None:
            acc = acc[:dh] / acc[dh:dh + 1]
        return m, acc

    hp = _H // 2

    def pair(j, m, last=False):
        qb, g = j // hp, j % hp
        m, o0 = step((2 * g + 1, qb, sb), (2 * g, sa, m))
        j1 = j + 1
        nxt = None if last else (2 * (j1 % hp), j1 // hp, sa)
        m, o1 = step(nxt, (2 * g + 1, sb, m))
        o_s[g, :, pl.ds(pl.multiple_of(qb * _NQ, _NQ), _NQ)] = (
            jnp.concatenate([o0, o1], axis=0))
        return m

    m, _ = step((0, 0, sa), None)
    m = jax.lax.fori_loop(0, nqb * hp - 1, pair, m)
    pair(nqb * hp - 1, m, last=True)

    for cp in late_cp:
        cp.wait()
    b1 = b1_v[...].astype(_F32).reshape(1, -1)
    b2 = b2_v[...].astype(_F32).reshape(1, -1)

    def attn_out(c):
        rows = pl.ds(c * _FC, _FC)
        o = o_s[:, :, rows].reshape(D, _FC).T.astype(_BF16)
        h = x_v[rows, :].astype(_F32) + _dot(o, wo_v[...])
        return h, _layernorm(h).astype(_BF16)

    nxt = attn_out(0)
    for c in range(nfc):
        h, hn = nxt
        a = _gelu(_dot(hn, w1_v[...]) + b1).astype(_BF16)
        if c + 1 < nfc:
            nxt = attn_out(c + 1)
        out_v[pl.ds(c * _FC, _FC), :] = (
            h + (_dot(a, w2_v[...]) + b2)).astype(out_v.dtype)
        out_cp[c].start()
    for cp in out_cp:
        cp.wait()


@jax.jit
def pallas_sequential_preLN__softmax_full_mha__dense_activation_gelu__prompt_kernel(
    A_x: jax.Array,
    A_wqkv: jax.Array,
    A_wo: jax.Array,
    B_x: jax.Array,
    B_w1: jax.Array,
    B_b1: jax.Array,
    B_w2: jax.Array,
    B_b2: jax.Array,
):
    del B_x
    _, S, D = A_x.shape
    F = B_w1.shape[1]
    dh = D // _H
    vm = -(-(dh + 1) // 8) * 8
    dt = A_x.dtype
    any_spec = pl.BlockSpec(memory_space=pl.ANY)
    return pl.pallas_call(
        _kernel,
        out_shape=jax.ShapeDtypeStruct(A_x.shape, dt),
        in_specs=[any_spec] * 7,
        out_specs=any_spec,
        scratch_shapes=[
            pltpu.VMEM((S, D), dt),
            pltpu.VMEM((D, D), dt),
            pltpu.VMEM((D, D), dt),
            pltpu.VMEM((D, D), dt),
            pltpu.VMEM((D, D), dt),
            pltpu.VMEM((D, F), dt),
            pltpu.VMEM((F,), dt),
            pltpu.VMEM((F, D), dt),
            pltpu.VMEM((D,), dt),
            pltpu.VMEM((S, D), dt),
            pltpu.VMEM((S, D), _BF16),
            pltpu.VMEM((S, D), _BF16),
            pltpu.VMEM((_H // 2, S, 2 * dh), _BF16),
            pltpu.VMEM((_H, 2 * dh, S), _BF16),
            pltpu.VMEM((_H, vm, S), _F32),
            pltpu.VMEM((S, _NQ), _F32),
            pltpu.VMEM((S, _NQ), _F32),
            pltpu.VMEM((_H // 2, 2 * dh, S), _F32),
            pltpu.SemaphoreType.DMA((S // _RC + 8 + S // _FC,)),
        ],
        compiler_params=pltpu.CompilerParams(vmem_limit_bytes=100 * 2**20),
    )(A_x, A_wqkv, A_wo, B_w1, B_b1, B_w2, B_b2)
```

```python
import math

import jax
import jax.numpy as jnp
import jax.experimental.pallas as pl
import jax.experimental.pallas.tpu as pltpu

_H = 32
_EPS = 1e-5
_RC = 512
_NQ = 512
_KC = 128
_FC = 256

_UNROLL = 4

_F32 = jnp.float32
_BF16 = jnp.bfloat16


def _dot(a, b):
    return jnp.dot(a, b, preferred_element_type=_F32)


def _dot_nt(a, b):
    return jax.lax.dot_general(
        a, b, (((1,), (1,)), ((), ())), preferred_element_type=_F32)


def _layernorm(x):
    d = x - jnp.mean(x, axis=-1, keepdims=True)
    v = jnp.mean(d * d, axis=-1, keepdims=True)
    return d * jax.lax.rsqrt(v + _EPS)


def _gelu(x):
    c = math.sqrt(2.0 / math.pi)
    return x * (0.5 * (1.0 + jnp.tanh(c * (x + 0.044715 * (x * x * x)))))


def _kernel(x_hbm, wqkv_hbm, wo_hbm, w1_hbm, b1_hbm, w2_hbm, b2_hbm, out_hbm,
            x_v, wk_v, wq_v, wv_v, wo_v, w1_v, b1_v, w2_v, b2_v, out_v,
            xn_s, kall_s, k_s, q_s, v_s, sa, sb, o_s, sems):
    S, D = x_v.shape
    dh = D // _H
    vm = v_s.shape[1]
    nrc, nqb, nkc, nfc = S // _RC, S // _NQ, S // _KC, S // _FC

    sem_id = iter(range(sems.shape[0]))

    def copy(src, dst):
        return pltpu.make_async_copy(src, dst, sems.at[next(sem_id)])

    x_cp = [copy(x_hbm.at[0, pl.ds(c * _RC, _RC)], x_v.at[pl.ds(c * _RC, _RC)])
            for c in range(nrc)]
    wq_cp = copy(wqkv_hbm.at[:, pl.ds(0, D)], wq_v)
    wk_cp = copy(wqkv_hbm.at[:, pl.ds(D, D)], wk_v)
    wv_cp = copy(wqkv_hbm.at[:, pl.ds(2 * D, D)], wv_v)
    late_cp = [copy(wo_hbm, wo_v), copy(w1_hbm, w1_v), copy(b1_hbm, b1_v),
               copy(w2_hbm, w2_v), copy(b2_hbm, b2_v)]
    out_cp = [copy(out_v.at[pl.ds(c * _FC, _FC)], out_hbm.at[0, pl.ds(c * _FC, _FC)])
              for c in range(nfc)]

    def norm(c):
        rows = pl.ds(c * _RC, _RC)
        xn = _layernorm(x_v[rows, :].astype(_F32)).astype(_BF16)
        xn_s[rows, :] = xn
        return xn

    x_cp[0].start()
    wk_cp.start()
    x_cp[0].wait()
    x_cp[1].start()
    xn = norm(0)
    wk_cp.wait()
    for cp in x_cp[2:] + [wq_cp, wv_cp]:
        cp.start()
    x_cp[1].wait()
    for c in range(nrc):
        if c == 1:
            for cp in x_cp[2:]:
                cp.wait()
        kall_s[pl.ds(c * _RC, _RC), :] = _dot(xn, wk_v[...]).astype(_BF16)
        if c + 1 < nrc:
            xn = norm(c + 1)
    wq_cp.wait()
    wv_cp.wait()
    for cp in late_cp:
        cp.start()
    wq_t = wq_v[...].T
    wv_t = wv_v[...].T
    qscale = dh ** -0.5 * math.log2(math.e)
    row = jax.lax.broadcasted_iota(jnp.int32, (vm - dh, _RC), 0)
    v_tail = jnp.where(row == 0, 1.0, 0.0).astype(_F32)
    first = jax.lax.broadcasted_iota(jnp.int32, (2 * dh, _RC), 0) < dh
    for c in range(nrc):
        cols = pl.ds(c * _RC, _RC)
        xn = xn_s[cols, :]
        qt = _dot_nt(wq_t, xn) * qscale
        vt = _dot_nt(wv_t, xn)
        k = kall_s[cols, :]
        for g in range(_H // 2):
            k_s[g, cols, :] = k[:, 2 * g * dh:2 * (g + 1) * dh]
            qg = qt[2 * g * dh:2 * (g + 1) * dh, :]
            q_s[2 * g, :, cols] = jnp.where(first, qg, 0.0).astype(_BF16)
            q_s[2 * g + 1, :, cols] = jnp.where(first, 0.0, qg).astype(_BF16)
        for h in range(_H):
            v_s[h, :, cols] = jnp.concatenate(
                [vt[h * dh:(h + 1) * dh, :], v_tail], axis=0)

    def step(nxt, cur):
        m = acc = None
        if nxt is not None:
            h1, qb1, s1 = nxt
            q = q_s[h1, :, pl.ds(pl.multiple_of(qb1 * _NQ, _NQ), _NQ)]
        if cur is not None:
            h0, s0, m0 = cur
        for c in range(nkc):
            keys = pl.ds(c * _KC, _KC)
            if nxt is not None:
                s = _dot(k_s[h1 // 2, keys, :], q)
                s1[keys, :] = s
                mm = jnp.max(s.reshape(_KC // 8, 8, _NQ), axis=0)
                m = mm if m is None else jnp.maximum(m, mm)
            if cur is not None:
                p = jnp.exp2(s0[keys, :] - m0).astype(_BF16)
                r = _dot(v_s[h0, :, keys], p)
                acc = r if acc is None else acc + r
        if m is not None:
            m = jnp.max(m, axis=0, keepdims=True)
        if acc is not None:
            acc = acc[:dh] / acc[dh:dh + 1]
        return m, acc

    hp = _H // 2

    def pair(j, m, last=False):
        qb, g = j // hp, j % hp
        m, o0 = step((2 * g + 1, qb, sb), (2 * g, sa, m))
        j1 = j + 1
        nxt = None if last else (2 * (j1 % hp), j1 // hp, sa)
        m, o1 = step(nxt, (2 * g + 1, sb, m))
        o_s[g, :, pl.ds(pl.multiple_of(qb * _NQ, _NQ), _NQ)] = (
            jnp.concatenate([o0, o1], axis=0))
        return m

    m, _ = step((0, 0, sa), None)

    def pairs(i, m):
        for u in range(_UNROLL):
            m = pair(i * _UNROLL + u, m)
        return m

    m = jax.lax.fori_loop(0, nqb * hp // _UNROLL - 1, pairs, m)
    for cp in late_cp:
        cp.wait()
    for j in range(nqb * hp - _UNROLL, nqb * hp):
        m = pair(j, m, last=j == nqb * hp - 1)

    b1 = b1_v[...].astype(_F32).reshape(1, -1)
    b2 = b2_v[...].astype(_F32).reshape(1, -1)

    def attn_out(c):
        rows = pl.ds(c * _FC, _FC)
        o = o_s[:, :, rows].reshape(D, _FC).T.astype(_BF16)
        h = x_v[rows, :].astype(_F32) + _dot(o, wo_v[...])
        return h, _layernorm(h).astype(_BF16)

    nxt = attn_out(0)
    for c in range(nfc):
        h, hn = nxt
        a = _gelu(_dot(hn, w1_v[...]) + b1).astype(_BF16)
        if c + 1 < nfc:
            nxt = attn_out(c + 1)
        out_v[pl.ds(c * _FC, _FC), :] = (
            h + (_dot(a, w2_v[...]) + b2)).astype(out_v.dtype)
        out_cp[c].start()
    for cp in out_cp:
        cp.wait()


@jax.jit
def pallas_sequential_preLN__softmax_full_mha__dense_activation_gelu__prompt_kernel(
    A_x: jax.Array,
    A_wqkv: jax.Array,
    A_wo: jax.Array,
    B_x: jax.Array,
    B_w1: jax.Array,
    B_b1: jax.Array,
    B_w2: jax.Array,
    B_b2: jax.Array,
):
    del B_x
    _, S, D = A_x.shape
    F = B_w1.shape[1]
    dh = D // _H
    vm = -(-(dh + 1) // 8) * 8
    dt = A_x.dtype
    any_spec = pl.BlockSpec(memory_space=pl.ANY)
    return pl.pallas_call(
        _kernel,
        out_shape=jax.ShapeDtypeStruct(A_x.shape, dt),
        in_specs=[any_spec] * 7,
        out_specs=any_spec,
        scratch_shapes=[
            pltpu.VMEM((S, D), dt),
            pltpu.VMEM((D, D), dt),
            pltpu.VMEM((D, D), dt),
            pltpu.VMEM((D, D), dt),
            pltpu.VMEM((D, D), dt),
            pltpu.VMEM((D, F), dt),
            pltpu.VMEM((F,), dt),
            pltpu.VMEM((F, D), dt),
            pltpu.VMEM((D,), dt),
            pltpu.VMEM((S, D), dt),
            pltpu.VMEM((S, D), _BF16),
            pltpu.VMEM((S, D), _BF16),
            pltpu.VMEM((_H // 2, S, 2 * dh), _BF16),
            pltpu.VMEM((_H, 2 * dh, S), _BF16),
            pltpu.VMEM((_H, vm, S), _F32),
            pltpu.VMEM((S, _NQ), _F32),
            pltpu.VMEM((S, _NQ), _F32),
            pltpu.VMEM((_H // 2, 2 * dh, S), _F32),
            pltpu.SemaphoreType.DMA((S // _RC + 8 + S // _FC,)),
        ],
        compiler_params=pltpu.CompilerParams(vmem_limit_bytes=100 * 2**20),
    )(A_x, A_wqkv, A_wo, B_w1, B_b1, B_w2, B_b2)
```
